```python
import jax
import jax.numpy as jnp

def _softmax(x, axis=-1):
    return jax.nn.softmax(x, axis=axis)
def _gelu(x):
    return jax.nn.gelu(x, approximate=True)
def _silu(x):
    return jax.nn.silu(x)
def _sigmoid(x):
    return jax.nn.sigmoid(x)
def _layernorm(x, axis=-1, eps=1e-5):
    m = jnp.mean(x, axis=axis, keepdims=True)
    v = jnp.var(x, axis=axis, keepdims=True)
    return (x - m) / jnp.sqrt(v + eps)
def _scatter_add(tgt, idx, src, axis=0):
    return tgt.at[idx].add(src)
def _segment_sum(src, seg, n):
    return jax.ops.segment_sum(src, seg, n)
class _Rng:
    def __init__(self, key):
        self._k = key
    def _next(self):
        self._k, sub = jax.random.split(self._k)
        return sub
    def normal(self, shape):
        return jax.random.normal(self._next(), shape, dtype=jnp.bfloat16)
    def randint(self, lo, hi, shape):
        return jax.random.randint(self._next(), shape, lo, hi, dtype=jnp.int32)
    def uniform(self, shape, lo=0.0, hi=1.0):
        return jax.random.uniform(self._next(), shape, jnp.bfloat16, lo, hi)
    def permutation(self, n):
        return jax.random.permutation(self._next(), n)


kernel_name = 'standalone__standard_2d_1d_3d_conv__vision'

def setup_inputs():
    _rng = _Rng(jax.random.key(int.from_bytes(__import__("os").urandom(4), "little")))
    _w = (lambda a: (lambda t: t.astype(jnp.bfloat16) if jnp.issubdtype(t.dtype, jnp.floating) else t)(jnp.asarray(a)))
    H = W = 384
    C = 384
    K = 1
    return {
        "x": _w((lambda *s: _rng.normal(s) * 0.05)(1, H, W, C)),
        "w": _w((lambda *s: _rng.normal(s) * 0.05)(K, K, C, C)),
        "b": _w((lambda *s: _rng.normal(s) * 0.05)(C)),
    }

def reference(x, w, b):
    B, H, W, Cin = x.shape
    K = w.shape[0]
    pl = (K - 1) // 2
    pr = K // 2
    xp = jnp.pad(x, ((0, 0), (pl, pr), (pl, pr), (0, 0)))
    out = sum(
        jnp.einsum('bhwc,cd->bhwd', xp[:, i:i+H, j:j+W, :], w[i, j])
        for i in range(K) for j in range(K)
    )
    return out + b[None, None, None, :]
```

```python
import jax
import jax.numpy as jnp
from jax import lax
import jax.experimental.pallas as pl
import jax.experimental.pallas.tpu as pltpu

_ROWS, _LANES = 8, 128
_PARTS = 3
_STREAM = 512
_UNIT = 6
_COLUMNS, _REST = divmod(_STREAM, _PARTS)

_CHUNK = 17
_AHEAD = 3
_RING = 4
_LEAD = 26
_LATE = 2
_WRITE_STEP = 32
_WRITE_PIECE = 2
_FIRST_WRITES = 8
_WRITE_RATE = 3


def _conv1x1_kernel(
    x_hbm, w_hbm, b_hbm, o_hbm, buf, w_ref, b_ref, ring, odd_sem, out_sem
):
    groups = buf.shape[0] // (2 * _UNIT)
    steps = _COLUMNS // _CHUNK
    step_tiles = _PARTS * _CHUNK
    n_reads = groups * steps
    unit_writes = _STREAM // _WRITE_STEP
    n_writes = 2 * groups * unit_writes
    switch = n_reads - _AHEAD

    def split(i, n):
        if isinstance(i, int):
            return divmod(i, n)
        q = lax.div(i, n)
        return q, i - q * n

    def window(src, dst, stream, streams, tile, tiles):
        row = tile * _ROWS
        if not isinstance(row, int):
            row = pl.multiple_of(row, _ROWS)
        idx = (pl.ds(stream, streams), pl.ds(row, tiles * _ROWS))
        src, dst = src.at[idx], dst.at[idx]

        def copy(offset, size, sem, thread):
            idx = (slice(None), pl.ds(offset * _ROWS, size * _ROWS))
            pltpu.make_async_copy(src.at[idx], dst.at[idx], sem).start(priority=thread)

        return copy

    def read_rest(stream, streams, sem, thread):
        copy = window(x_hbm, buf, stream, streams, _STREAM - _REST, _REST)
        copy(0, _REST, sem, thread)

    def wait(tiles, sem):
        full, part = divmod(tiles, _STREAM)
        if full:
            size = buf.at[pl.ds(0, full)]
            pltpu.make_async_copy(size, size, sem).wait()
        if part:
            size = buf.at[pl.ds(0, 1), pl.ds(0, part * _ROWS)]
            pltpu.make_async_copy(size, size, sem).wait()

    def read_odd(n):
        g, column = divmod(n, _COLUMNS)
        if g < groups:
            stream, tile = (2 * g + 1) * _UNIT, column * _PARTS
            window(x_hbm, buf, stream, _UNIT, tile, _PARTS)(0, _PARTS, odd_sem, 1)
        else:
            g, pair = divmod(column, _UNIT // 2)
            read_rest((2 * g + 1) * _UNIT + 2 * pair, 2, odd_sem, 1)

    n_odd = groups * (_COLUMNS + _UNIT // 2)

    def read_step(i):
        g, j = split(i, steps)
        sem = ring.at[i & (_RING - 1)]
        even = window(x_hbm, buf, 2 * g * _UNIT, _UNIT, j * step_tiles, step_tiles)
        if isinstance(i, int):
            assert j > 0
            for c in range(_CHUNK):
                late = i == n_reads - 1 and c >= _CHUNK - _LATE
                even(c * _PARTS, _PARTS, odd_sem if late else sem, 0)
                read_odd(i * _CHUNK + c + _LEAD)
            return

        @pl.when(j == 0)
        def _():
            read_rest(2 * g * _UNIT, _UNIT, sem, 0)

        odd = []
        for later in range(2):
            g1, j1 = split(i + _LEAD // _CHUNK + later, steps)
            stream = (2 * g1 + 1) * _UNIT
            odd.append(window(x_hbm, buf, stream, _UNIT, j1 * step_tiles, step_tiles))
        for c in range(_CHUNK):
            even(c * _PARTS, _PARTS, sem, 0)
            later, c1 = divmod(c + _LEAD % _CHUNK, _CHUNK)
            odd[later](c1 * _PARTS, _PARTS, odd_sem, 1)

    def unit_of(v):
        return jnp.where(v < groups, 2 * v, 2 * (v - groups) + 1)

    def write_steps(lo, hi):
        def body(s, carry):
            v = s >> (unit_writes.bit_length() - 1)
            tile = (s & (unit_writes - 1)) * _WRITE_STEP
            copy = window(buf, o_hbm, unit_of(v) * _UNIT, _UNIT, tile, _WRITE_STEP)
            for t in range(0, _WRITE_STEP, _WRITE_PIECE):
                copy(t, _WRITE_PIECE, out_sem, 1)
            return carry

        lax.fori_loop(lo, hi, body, 0)

    def matmul(view, pixels):
        def at(stream, tile):
            return stream, pl.ds(tile * _ROWS, _ROWS), slice(None)

        lhs = jnp.concatenate(
            [
                jnp.concatenate([view[at(*tiles[part])] for tiles in pixels])
                for part in range(_PARTS)
            ],
            axis=1,
        )
        acc = jnp.dot(lhs, w_ref[...], preferred_element_type=jnp.float32)
        out = (acc + bias).astype(buf.dtype)
        for q, tiles in enumerate(pixels):
            for part in range(_PARTS):
                view[at(*tiles[part])] = out[
                    q * _ROWS:(q + 1) * _ROWS, part * _LANES:(part + 1) * _LANES
                ]

    def compute(unit, j):
        first = [-s * _STREAM % _PARTS for s in range(_UNIT)]
        streams = pl.ds(unit * _UNIT, _UNIT)

        @pl.when(j == 0)
        def _():
            matmul(buf.at[streams], [
                [divmod(s * _STREAM + first[s] - _PARTS + t, _STREAM) for t in range(_PARTS)]
                for s in range(_UNIT) if first[s]
            ])

        row = pl.multiple_of(j * (step_tiles * _ROWS), _ROWS)
        view = buf.at[streams, pl.ds(row, (step_tiles + _REST) * _ROWS)]
        matmul(view, [
            [(s, first[s] + c * _PARTS + t) for t in range(_PARTS)]
            for s in range(_UNIT) for c in range(_CHUNK)
        ])

    for n in range(_LEAD):
        read_odd(n)
    w_copy = pltpu.make_async_copy(w_hbm, w_ref, out_sem)
    b_copy = pltpu.make_async_copy(b_hbm, b_ref, out_sem)
    w_copy.start()
    b_copy.start()

    def prologue(i, carry):
        read_step(i)
        return carry

    lax.fori_loop(0, _AHEAD, prologue, 0)
    w_copy.wait()
    b_copy.wait()
    bias = b_ref[...].astype(jnp.float32).reshape(1, _PARTS * _LANES)
    wait(_UNIT * (step_tiles + _REST), ring.at[0])

    unrolled = (groups * _COLUMNS - _LEAD) // _CHUNK

    def writes_after(done):
        return _FIRST_WRITES + (done - switch) * _WRITE_RATE

    for done in range(switch, 2 * n_reads):
        v, tile = divmod(writes_after(done) * _WRITE_STEP - 1, _STREAM)
        assert v * steps + min(tile // step_tiles, steps - 1) < done

    def step(i, carry):
        v, j = split(i, steps)

        @pl.when(i + _AHEAD < unrolled)
        def _():
            read_step(i + _AHEAD)

        for last in range(unrolled, n_reads):

            @pl.when(i + _AHEAD == last)
            def _():
                read_step(last)
                if last == n_reads - 1:
                    for n in range(n_reads * _CHUNK + _LEAD, n_odd):
                        read_odd(n)

        @pl.when(i < switch)
        def _():
            sem = ring.at[(i + 1) & (_RING - 1)]
            wait(_UNIT * step_tiles, sem)
            pl.when(j == steps - 1)(lambda: wait(_UNIT * _REST, sem))

        @pl.when(i == switch)
        def _():
            late = _UNIT * _PARTS * _LATE
            for t in range(switch + 1, n_reads):
                tiles = _UNIT * step_tiles - (late if t == n_reads - 1 else 0)
                wait(tiles, ring.at[t % _RING])
            write_steps(0, _FIRST_WRITES)
            wait(groups * _UNIT * _STREAM + late, odd_sem)

        compute(unit_of(v), j)

        @pl.when(i >= switch)
        def _():
            hi = jnp.where(i == 2 * n_reads - 1, n_writes, writes_after(i + 1))
            write_steps(writes_after(i), hi)

        return carry

    lax.fori_loop(0, 2 * n_reads, step, 0)
    pltpu.make_async_copy(buf, o_hbm, out_sem).wait()


@jax.jit
def pallas_standalone__standard_2d_1d_3d_conv__vision_kernel(
    x: jax.Array,
    w: jax.Array,
    b: jax.Array,
):
    batch, height, width, cin = x.shape
    kh, kw, _, cout = w.shape
    groups_of_8 = batch * height * width // _ROWS
    streams = groups_of_8 * _PARTS // _STREAM
    assert (kh, kw) == (1, 1) and cin == cout == _PARTS * _LANES
    assert streams * _STREAM * _ROWS * _LANES == x.size
    assert streams % (2 * _UNIT) == 0
    shape = (streams, _STREAM * _ROWS, _LANES)
    tiles = x.reshape(groups_of_8, _ROWS, _PARTS, _LANES).transpose(0, 2, 1, 3)
    hbm = pl.BlockSpec(memory_space=pltpu.HBM)
    out = pl.pallas_call(
        _conv1x1_kernel,
        in_specs=[hbm, hbm, hbm],
        out_specs=hbm,
        out_shape=jax.ShapeDtypeStruct(shape, x.dtype),
        scratch_shapes=[
            pltpu.VMEM(shape, x.dtype),
            pltpu.VMEM((cin, cout), w.dtype),
            pltpu.VMEM((cout,), b.dtype),
            pltpu.SemaphoreType.DMA((_RING,)),
            pltpu.SemaphoreType.DMA(()),
            pltpu.SemaphoreType.DMA(()),
        ],
        compiler_params=pltpu.CompilerParams(
            vmem_limit_bytes=120 * 2**20,
            disable_bounds_checks=True,
            disable_semaphore_checks=True,
        ),
    )(tiles.reshape(shape), w.reshape(cin, cout), b)
    out = out.reshape(groups_of_8, _PARTS, _ROWS, _LANES).transpose(0, 2, 1, 3)
    return out.reshape(batch, height, width, cout)
```

```python
import jax
import jax.numpy as jnp
from jax import lax
import jax.experimental.pallas as pl
import jax.experimental.pallas.tpu as pltpu

_ROWS, _LANES = 8, 128
_PARTS = 3
_STREAM = 512
_UNIT = 6
_COLUMNS, _REST = divmod(_STREAM, _PARTS)

_CHUNK = 17
_AHEAD = 3
_RING = 4
_LEAD = 26
_WEIGHT_TURNS = 4
_LATE = 2
_WRITE_STEP = 32
_WRITE_PIECE = 4
_FIRST_WRITES = 8
_WRITE_RATE = 3


def _conv1x1_kernel(
    x_hbm, w_hbm, b_hbm, o_hbm, buf, w_ref, b_ref, ring, odd_sem, out_sem
):
    groups = buf.shape[0] // (2 * _UNIT)
    steps = _COLUMNS // _CHUNK
    step_tiles = _PARTS * _CHUNK
    n_reads = groups * steps
    unit_writes = _STREAM // _WRITE_STEP
    n_writes = 2 * groups * unit_writes
    n_odd = groups * (_COLUMNS + _UNIT // 2)
    switch = n_reads - _AHEAD

    def split(i, n):
        if isinstance(i, int):
            return divmod(i, n)
        q = lax.div(i, n)
        return q, i - q * n

    def window(src, dst, stream, streams, tile, tiles):
        row = tile * _ROWS
        if not isinstance(row, int):
            row = pl.multiple_of(row, _ROWS)
        idx = (pl.ds(stream, streams), pl.ds(row, tiles * _ROWS))
        src, dst = src.at[idx], dst.at[idx]

        def copy(offset, size, sem, thread):
            idx = (slice(None), pl.ds(offset * _ROWS, size * _ROWS))
            pltpu.make_async_copy(src.at[idx], dst.at[idx], sem).start(priority=thread)

        return copy

    def read_rest(stream, streams, sem, thread):
        copy = window(x_hbm, buf, stream, streams, _STREAM - _REST, _REST)
        copy(0, _REST, sem, thread)

    def wait(tiles, sem):
        full, part = divmod(tiles, _STREAM)
        if full:
            size = buf.at[pl.ds(0, full)]
            pltpu.make_async_copy(size, size, sem).wait()
        if part:
            size = buf.at[pl.ds(0, 1), pl.ds(0, part * _ROWS)]
            pltpu.make_async_copy(size, size, sem).wait()

    def read_odd(n):
        g, column = divmod(n, _COLUMNS)
        if g < groups:
            stream, tile = (2 * g + 1) * _UNIT, column * _PARTS
            window(x_hbm, buf, stream, _UNIT, tile, _PARTS)(0, _PARTS, odd_sem, 1)
        elif n < n_odd:
            g, pair = divmod(n - groups * _COLUMNS, _UNIT // 2)
            read_rest((2 * g + 1) * _UNIT + 2 * pair, 2, odd_sem, 1)

    def read_step(i):
        g, j = split(i, steps)
        sem = ring.at[i & (_RING - 1)]
        even = window(x_hbm, buf, 2 * g * _UNIT, _UNIT, j * step_tiles, step_tiles)
        if isinstance(i, int):
            assert j > 0
            for c in range(_CHUNK):
                late = i == n_reads - 1 and c >= _CHUNK - _LATE
                even(c * _PARTS, _PARTS, odd_sem if late else sem, 0)
                read_odd(i * _CHUNK + c + _LEAD)
            return

        @pl.when(j == 0)
        def _():
            read_rest(2 * g * _UNIT, _UNIT, sem, 0)

        odd = []
        for later in range(2):
            g1, j1 = split(i + _LEAD // _CHUNK + later, steps)
            stream = (2 * g1 + 1) * _UNIT
            odd.append(window(x_hbm, buf, stream, _UNIT, j1 * step_tiles, step_tiles))
        for c in range(_CHUNK):
            even(c * _PARTS, _PARTS, sem, 0)
            later, c1 = divmod(c + _LEAD % _CHUNK, _CHUNK)
            odd[later](c1 * _PARTS, _PARTS, odd_sem, 1)

    def unit_of(v):
        return jnp.where(v < groups, 2 * v, 2 * (v - groups) + 1)

    def write_steps(lo, hi):
        def body(s, carry):
            v = s >> (unit_writes.bit_length() - 1)
            tile = (s & (unit_writes - 1)) * _WRITE_STEP
            copy = window(buf, o_hbm, unit_of(v) * _UNIT, _UNIT, tile, _WRITE_STEP)
            for t in range(0, _WRITE_STEP, _WRITE_PIECE):
                copy(t, _WRITE_PIECE, out_sem, 1)
            return carry

        lax.fori_loop(lo, hi, body, 0)

    def matmul(view, pixels):
        def at(stream, tile):
            return stream, pl.ds(tile * _ROWS, _ROWS), slice(None)

        lhs = jnp.concatenate(
            [
                jnp.concatenate([view[at(*tiles[part])] for tiles in pixels])
                for part in range(_PARTS)
            ],
            axis=1,
        )
        acc = jnp.dot(lhs, w_ref[...], preferred_element_type=jnp.float32)
        out = (acc + bias).astype(buf.dtype)
        for q, tiles in enumerate(pixels):
            for part in range(_PARTS):
                view[at(*tiles[part])] = out[
                    q * _ROWS:(q + 1) * _ROWS, part * _LANES:(part + 1) * _LANES
                ]

    def compute(unit, j):
        first = [-s * _STREAM % _PARTS for s in range(_UNIT)]
        streams = pl.ds(unit * _UNIT, _UNIT)

        @pl.when(j == 0)
        def _():
            matmul(buf.at[streams], [
                [divmod(s * _STREAM + first[s] - _PARTS + t, _STREAM) for t in range(_PARTS)]
                for s in range(_UNIT) if first[s]
            ])

        row = pl.multiple_of(j * (step_tiles * _ROWS), _ROWS)
        view = buf.at[streams, pl.ds(row, (step_tiles + _REST) * _ROWS)]
        matmul(view, [
            [(s, first[s] + c * _PARTS + t) for t in range(_PARTS)]
            for s in range(_UNIT) for c in range(_CHUNK)
        ])

    def read_weights(turn, thread):
        rows = w_ref.shape[0] // (2 * _WEIGHT_TURNS)
        rows = pl.ds((2 * turn + thread) * rows, rows)
        copy = pltpu.make_async_copy(w_hbm.at[rows], w_ref.at[rows], out_sem)
        copy.start(priority=thread)

    for turn in range(_WEIGHT_TURNS):
        read_weights(turn, 1)
    for n in range(_LEAD):
        if n >= _LEAD - _WEIGHT_TURNS:
            read_weights(n - _LEAD + _WEIGHT_TURNS, 0)
        read_odd(n)
    b_copy = pltpu.make_async_copy(b_hbm, b_ref, out_sem)
    b_copy.start()

    def prologue(i, carry):
        read_step(i)
        return carry

    lax.fori_loop(0, _AHEAD, prologue, 0)
    pltpu.make_async_copy(w_hbm, w_ref, out_sem).wait()
    b_copy.wait()
    bias = b_ref[...].astype(jnp.float32).reshape(1, _PARTS * _LANES)
    wait(_UNIT * (step_tiles + _REST), ring.at[0])

    unrolled = (groups * _COLUMNS - _LEAD) // _CHUNK

    def writes_after(done):
        return _FIRST_WRITES + (done - switch) * _WRITE_RATE

    for done in range(switch, 2 * n_reads):
        v, tile = divmod(writes_after(done) * _WRITE_STEP - 1, _STREAM)
        assert v * steps + min(tile // step_tiles, steps - 1) < done
        assert writes_after(done) <= n_writes

    def step(i, carry):
        v, j = split(i, steps)

        @pl.when(i + _AHEAD < unrolled)
        def _():
            read_step(i + _AHEAD)

        for last in range(unrolled, n_reads):

            @pl.when(i + _AHEAD == last)
            def _():
                read_step(last)
                if last == n_reads - 1:
                    for n in range(n_reads * _CHUNK + _LEAD, n_odd):
                        read_odd(n)

        @pl.when(i < switch)
        def _():
            sem = ring.at[(i + 1) & (_RING - 1)]
            wait(_UNIT * step_tiles, sem)
            pl.when(j == steps - 1)(lambda: wait(_UNIT * _REST, sem))

        @pl.when(i == switch)
        def _():
            late = _UNIT * _PARTS * _LATE
            for t in range(switch + 1, n_reads):
                tiles = _UNIT * step_tiles - (late if t == n_reads - 1 else 0)
                wait(tiles, ring.at[t % _RING])
            write_steps(0, _FIRST_WRITES)
            wait(groups * _UNIT * _STREAM + late, odd_sem)

        compute(unit_of(v), j)

        @pl.when(i >= switch)
        def _():
            hi = jnp.where(i == 2 * n_reads - 1, n_writes, writes_after(i + 1))
            write_steps(writes_after(i), hi)

        return carry

    lax.fori_loop(0, 2 * n_reads, step, 0)
    pltpu.make_async_copy(buf, o_hbm, out_sem).wait()


@jax.jit
def pallas_standalone__standard_2d_1d_3d_conv__vision_kernel(
    x: jax.Array,
    w: jax.Array,
    b: jax.Array,
):
    batch, height, width, cin = x.shape
    kh, kw, _, cout = w.shape
    groups_of_8 = batch * height * width // _ROWS
    streams = groups_of_8 * _PARTS // _STREAM
    assert (kh, kw) == (1, 1) and cin == cout == _PARTS * _LANES
    assert streams * _STREAM * _ROWS * _LANES == x.size
    assert streams % (2 * _UNIT) == 0
    shape = (streams, _STREAM * _ROWS, _LANES)
    tiles = x.reshape(groups_of_8, _ROWS, _PARTS, _LANES).transpose(0, 2, 1, 3)
    hbm = pl.BlockSpec(memory_space=pltpu.HBM)
    out = pl.pallas_call(
        _conv1x1_kernel,
        in_specs=[hbm, hbm, hbm],
        out_specs=hbm,
        out_shape=jax.ShapeDtypeStruct(shape, x.dtype),
        scratch_shapes=[
            pltpu.VMEM(shape, x.dtype),
            pltpu.VMEM((cin, cout), w.dtype),
            pltpu.VMEM((cout,), b.dtype),
            pltpu.SemaphoreType.DMA((_RING,)),
            pltpu.SemaphoreType.DMA(()),
            pltpu.SemaphoreType.DMA(()),
        ],
        compiler_params=pltpu.CompilerParams(
            vmem_limit_bytes=120 * 2**20,
            disable_bounds_checks=True,
            disable_semaphore_checks=True,
        ),
    )(tiles.reshape(shape), w.reshape(cin, cout), b)
    out = out.reshape(groups_of_8, _PARTS, _ROWS, _LANES).transpose(0, 2, 1, 3)
    return out.reshape(batch, height, width, cout)
```

```python
import jax
import jax.numpy as jnp
from jax import lax
import jax.experimental.pallas as pl
import jax.experimental.pallas.tpu as pltpu

_ROWS, _LANES = 8, 128
_PARTS = 3
_STREAM = 512
_UNIT = 6
_PIECE = 8
_PAIR = 2

_CHUNK = 51
_AHEAD = 2
_RING = 4
_LEAD = 9
_LATE = 3
_WEIGHT_TURNS = 6
_WRITE_STEP = 32
_FIRST_WRITES = 8
_WRITE_RATE = 3


def _conv1x1_kernel(
    x_hbm, w_hbm, b_hbm, o_hbm, buf, w_ref, b_ref, ring, odd_sem, out_sem
):
    groups = buf.shape[0] // (2 * _UNIT)
    steps, rest = divmod(_STREAM, _CHUNK)
    pieces = _STREAM // _PIECE
    turns = _UNIT // _PAIR
    n_reads = groups * steps
    switch = n_reads - _AHEAD
    unit_writes = _STREAM // _WRITE_STEP
    n_writes = 2 * groups * unit_writes

    def split(i, n):
        if isinstance(i, int):
            return divmod(i, n)
        if n & (n - 1) == 0:
            return i >> (n.bit_length() - 1), i & (n - 1)
        q = lax.div(i, n)
        return q, i - q * n

    def window(src, dst, unit, tile, tiles):
        row = tile * _ROWS
        if not isinstance(row, int):
            row = pl.multiple_of(row, _ROWS)
        idx = (pl.ds(unit * _UNIT, _UNIT), pl.ds(row, tiles * _ROWS))
        src, dst = src.at[idx], dst.at[idx]

        def copy(stream, streams, tile, tiles, sem, thread):
            idx = (pl.ds(stream, streams), pl.ds(tile * _ROWS, tiles * _ROWS))
            pltpu.make_async_copy(src.at[idx], dst.at[idx], sem).start(priority=thread)

        return copy

    def wait(tiles, sem):
        full, part = divmod(tiles, _STREAM)
        if full:
            size = buf.at[pl.ds(0, full)]
            pltpu.make_async_copy(size, size, sem).wait()
        if part:
            size = buf.at[pl.ds(0, 1), pl.ds(0, part * _ROWS)]
            pltpu.make_async_copy(size, size, sem).wait()

    def reader(n, thread):
        g, piece = split(n, pieces)
        return window(x_hbm, buf, 2 * g + thread, piece * _PIECE, _PIECE)

    def pieces_after(j):
        n = (j * _CHUNK + rest + _PIECE - 1) >> (_PIECE.bit_length() - 1)
        return n if isinstance(j, int) else jnp.where(j == 0, 0, n)

    small = _LEAD // 3
    whole = groups * pieces - small
    unrolled = (groups - 1) * steps + next(
        j for j in range(steps, 0, -1)
        if (groups - 1) * pieces + pieces_after(j) + _LEAD <= whole
    )

    def read_step(i):
        g, j = split(i, steps)
        sem = ring.at[i & (_RING - 1)]
        lo, hi = g * pieces + pieces_after(j), g * pieces + pieces_after(j + 1)

        if isinstance(i, int):
            for n in range(lo, hi):
                even = reader(n, 0)
                for t in range(turns):
                    left = (groups * pieces - n) * turns - t
                    even_sem = odd_sem if left <= _LATE else sem
                    even(t * _PAIR, _PAIR, 0, _PIECE, even_sem, 0)
                    if n + _LEAD < whole:
                        reader(n + _LEAD, 1)(t * _PAIR, _PAIR, 0, _PIECE, odd_sem, 1)
                    else:
                        q, half = divmod((n + _LEAD - whole) * turns + t, 2)
                        q, stream = divmod(q, _UNIT)
                        size = _PIECE // 2
                        reader(whole + q, 1)(stream, 1, half * size, size, odd_sem, 1)
            return

        def body(n, carry):
            even, odd = reader(n, 0), reader(n + _LEAD, 1)
            for t in range(turns):
                even(t * _PAIR, _PAIR, 0, _PIECE, sem, 0)
                odd(t * _PAIR, _PAIR, 0, _PIECE, odd_sem, 1)
            return carry

        lax.fori_loop(lo, hi, body, 0)

    def wait_step(i):
        _, j = split(i, steps)
        sem = ring.at[i & (_RING - 1)]
        n = pieces_after(j + 1) - pieces_after(j)
        if isinstance(i, int):
            late = _LATE * _PAIR * _PIECE if i == n_reads - 1 else 0
            wait(n * _UNIT * _PIECE - late, sem)
        else:
            least = _CHUNK // _PIECE
            wait(least * _UNIT * _PIECE, sem)
            pl.when(n > least)(lambda: wait(_UNIT * _PIECE, sem))

    def unit_of(v):
        return jnp.where(v < groups, 2 * v, 2 * (v - groups) + 1)

    def write_steps(lo, hi):
        def body(s, carry):
            v, r = split(s, unit_writes)
            copy = window(buf, o_hbm, unit_of(v), r * _WRITE_STEP, _WRITE_STEP)
            for t in range(0, _WRITE_STEP, _PIECE):
                copy(0, _UNIT, t, _PIECE, out_sem, 1)
            return carry

        lax.fori_loop(lo, hi, body, 0)

    def matmul(view, pixels):
        def at(stream, tile):
            return stream, pl.ds(tile * _ROWS, _ROWS), slice(None)

        lhs = jnp.concatenate(
            [
                jnp.concatenate([view[at(*tiles[part])] for tiles in pixels])
                for part in range(_PARTS)
            ],
            axis=1,
        )
        acc = jnp.dot(lhs, w_ref[...], preferred_element_type=jnp.float32)
        out = (acc + bias).astype(buf.dtype)
        for q, tiles in enumerate(pixels):
            for part in range(_PARTS):
                view[at(*tiles[part])] = out[
                    q * _ROWS:(q + 1) * _ROWS, part * _LANES:(part + 1) * _LANES
                ]

    def compute(v, j):
        first = [-s * _STREAM % _PARTS for s in range(_UNIT)]
        streams = pl.ds(unit_of(v) * _UNIT, _UNIT)

        @pl.when(j == jnp.where(v < groups, steps - 1, 0))
        def _():
            matmul(buf.at[streams], [
                [divmod(s * _STREAM + first[s] - _PARTS + t, _STREAM) for t in range(_PARTS)]
                for s in range(_UNIT) if first[s]
            ])

        row = pl.multiple_of(j * (_CHUNK * _ROWS), _ROWS)
        view = buf.at[streams, pl.ds(row, (_CHUNK + rest) * _ROWS)]
        matmul(view, [
            [(s, first[s] + c + t) for t in range(_PARTS)]
            for s in range(_UNIT) for c in range(0, _CHUNK, _PARTS)
        ])

    def read_weights(turn, thread):
        rows = w_ref.shape[0] // (2 * _WEIGHT_TURNS)
        rows = pl.ds((2 * turn + thread) * rows, rows)
        copy = pltpu.make_async_copy(w_hbm.at[rows], w_ref.at[rows], out_sem)
        copy.start(priority=thread)

    for turn in range(_WEIGHT_TURNS):
        read_weights(turn, 1)
    for turn in range(_LEAD * turns):
        if turn >= _LEAD * turns - _WEIGHT_TURNS:
            read_weights(turn - _LEAD * turns + _WEIGHT_TURNS, 0)
        n, t = divmod(turn, turns)
        reader(n, 1)(t * _PAIR, _PAIR, 0, _PIECE, odd_sem, 1)
    b_copy = pltpu.make_async_copy(b_hbm, b_ref, out_sem)
    b_copy.start()

    def prologue(i, carry):
        read_step(i)
        return carry

    lax.fori_loop(0, _AHEAD, prologue, 0)
    pltpu.make_async_copy(w_hbm, w_ref, out_sem).wait()
    b_copy.wait()
    bias = b_ref[...].astype(jnp.float32).reshape(1, _PARTS * _LANES)

    def writes_after(done):
        return _FIRST_WRITES + (done - switch) * _WRITE_RATE

    for done in range(switch, 2 * n_reads):
        v, tile = divmod(writes_after(done) * _WRITE_STEP - 1, _STREAM)
        assert v * steps + min(tile // _CHUNK, steps - 1) < done
        assert writes_after(done) <= n_writes

    def step(i, carry):
        @pl.when(i + _AHEAD < unrolled)
        def _():
            read_step(i + _AHEAD)

        for last in range(unrolled, n_reads):
            pl.when(i + _AHEAD == last)(lambda: read_step(last))

        pl.when(i < switch)(lambda: wait_step(i))

        @pl.when(i == switch)
        def _():
            for t in range(switch, n_reads):
                wait_step(t)
            write_steps(0, _FIRST_WRITES)
            wait(groups * _UNIT * _STREAM + _LATE * _PAIR * _PIECE, odd_sem)

        compute(*split(i, steps))

        @pl.when(i >= switch)
        def _():
            hi = jnp.where(i == 2 * n_reads - 1, n_writes, writes_after(i + 1))
            write_steps(writes_after(i), hi)

        return carry

    lax.fori_loop(0, 2 * n_reads, step, 0)
    pltpu.make_async_copy(buf, o_hbm, out_sem).wait()


@jax.jit
def pallas_standalone__standard_2d_1d_3d_conv__vision_kernel(
    x: jax.Array,
    w: jax.Array,
    b: jax.Array,
):
    batch, height, width, cin = x.shape
    kh, kw, _, cout = w.shape
    groups_of_8 = batch * height * width // _ROWS
    streams = groups_of_8 * _PARTS // _STREAM
    assert (kh, kw) == (1, 1) and cin == cout == _PARTS * _LANES
    assert streams * _STREAM * _ROWS * _LANES == x.size
    assert streams % (2 * _UNIT) == 0
    shape = (streams, _STREAM * _ROWS, _LANES)
    tiles = x.reshape(groups_of_8, _ROWS, _PARTS, _LANES).transpose(0, 2, 1, 3)
    hbm = pl.BlockSpec(memory_space=pltpu.HBM)
    out = pl.pallas_call(
        _conv1x1_kernel,
        in_specs=[hbm, hbm, hbm],
        out_specs=hbm,
        out_shape=jax.ShapeDtypeStruct(shape, x.dtype),
        scratch_shapes=[
            pltpu.VMEM(shape, x.dtype),
            pltpu.VMEM((cin, cout), w.dtype),
            pltpu.VMEM((cout,), b.dtype),
            pltpu.SemaphoreType.DMA((_RING,)),
            pltpu.SemaphoreType.DMA(()),
            pltpu.SemaphoreType.DMA(()),
        ],
        compiler_params=pltpu.CompilerParams(
            vmem_limit_bytes=120 * 2**20,
            disable_bounds_checks=True,
            disable_semaphore_checks=True,
        ),
    )(tiles.reshape(shape), w.reshape(cin, cout), b)
    out = out.reshape(groups_of_8, _PARTS, _ROWS, _LANES).transpose(0, 2, 1, 3)
    return out.reshape(batch, height, width, cout)
```

```python
import jax
import jax.numpy as jnp
from jax import lax
import jax.experimental.pallas as pl
import jax.experimental.pallas.tpu as pltpu

_ROWS, _LANES = 8, 128
_PARTS = 3
_STREAM = 512
_UNIT = 6
_PIECE = 8
_CHUNK = 51

_PAIR = 2
_READ_STEP = 16
_FIRST_READS = 8
_READ_RATE = 53
_RING = 32
_LEAD = 26
_WEIGHT_TURNS = 6

_LATE = 5
_WRITE_STEP = 32
_FIRST_WRITES = 8
_WRITE_RATE = 46


def _split(i, n):
    if isinstance(i, int):
        return divmod(i, n)
    if n & (n - 1) == 0:
        return i >> (n.bit_length() - 1), i & (n - 1)
    q = lax.div(i, n)
    return q, i - q * n


def _window(src, dst, stream, streams, tile, tiles):
    row = tile * _ROWS
    if not isinstance(row, int):
        row = pl.multiple_of(row, _ROWS)
    idx = (pl.ds(stream, streams), pl.ds(row, tiles * _ROWS))
    src, dst = src.at[idx], dst.at[idx]

    def copy(stream, streams, tile, tiles, sem, thread):
        idx = (pl.ds(stream, streams), pl.ds(tile * _ROWS, tiles * _ROWS))
        pltpu.make_async_copy(src.at[idx], dst.at[idx], sem).start(priority=thread)

    return copy


def _conv1x1_kernel(
    x_hbm, w_hbm, b_hbm, o_hbm, buf, w_ref, b_ref, ring, odd_sem, last_sem, out_sem
):
    groups = buf.shape[0] // (2 * _UNIT)
    chunks, rest = divmod(_STREAM, _CHUNK)
    n_matmuls = 2 * groups * chunks
    group_reads = _STREAM // _READ_STEP
    n_reads = groups * group_reads
    unit_writes = _STREAM // _WRITE_STEP
    n_writes = 2 * groups * unit_writes

    def wait(tiles, sem):
        full, part = divmod(tiles, _STREAM)
        if full:
            size = buf.at[pl.ds(0, full)]
            pltpu.make_async_copy(size, size, sem).wait()
        if part:
            size = buf.at[pl.ds(0, 1), pl.ds(0, part * _ROWS)]
            pltpu.make_async_copy(size, size, sem).wait()

    def unit_of(v):
        return jnp.where(v < groups, 2 * v, 2 * (v - groups) + 1)

    pairs = 2 * _UNIT // _PAIR
    step_copies = pairs * _READ_STEP // _PIECE
    n_copies = n_reads * step_copies
    first_cut = n_copies + 1 - 2 * pl.cdiv(_LEAD, 3)
    unrolled = (first_cut - 2 * _LEAD) // step_copies
    last_even = range(unrolled * step_copies, n_copies, 2)
    on_time = last_even[:len(last_even) - _LATE]

    def reader(m):
        g, r = _split(m, group_reads)
        stream, tile = 2 * g * _UNIT, r * _READ_STEP
        copy = _window(x_hbm, buf, stream, 2 * _UNIT, tile, _READ_STEP)
        even_sem = ring.at[m & (_RING - 1)]

        def read(c, sem=None, quarter=None):
            piece, pair = divmod(c, pairs)
            stream, tile = pair * _PAIR, piece * _PIECE
            if sem is None:
                sem = even_sem if stream < _UNIT else odd_sem
            if quarter is None:
                copy(stream, _PAIR, tile, _PIECE, sem, c % 2)
            else:
                s, half = divmod(quarter, 2)
                copy(stream + s, 1, tile + half * _PIECE // 2, _PIECE // 2, sem, c % 2)

        return read

    def read(c, *args):
        m, c = divmod(c, step_copies)
        reader(m)(c, *args)

    def read_step(m, carry):
        readers = {}
        for c in range(step_copies):
            later, c = divmod(c + c % 2 * 2 * _LEAD, step_copies)
            if later not in readers:
                readers[later] = reader(m + later)
            readers[later](c)
        return carry

    def read_last_steps():
        odd = [(c,) for c in range(last_even[0] + 2 * _LEAD + 1, first_cut, 2)]
        odd += [(c, q) for c in range(first_cut, n_copies, 2) for q in range(4)]
        for turn, (c, *quarter) in enumerate(odd):
            if turn < len(last_even):
                even = last_even[turn]
                read(even, last_sem if even in on_time else odd_sem)
            read(c, odd_sem, *quarter)

    def reads_needed(done):
        g, j = _split(done, chunks)
        n, _ = _split(j * _CHUNK + rest + _READ_STEP - 1, _READ_STEP)
        n = n * (j > 0) if isinstance(done, int) else jnp.where(j > 0, n, 0)
        return g * group_reads + n

    def wait_step(m, carry):
        wait(_UNIT * _READ_STEP, ring.at[m & (_RING - 1)])
        return carry

    def wait_last_steps(first):
        left = buf.shape[0] * _STREAM - first * _UNIT * _READ_STEP
        left -= len(on_time) * _PAIR * _PIECE
        for m in range(first, n_reads):
            copies = [
                c for c in range(m * step_copies, (m + 1) * step_copies)
                if c % pairs * _PAIR < _UNIT and c - c % 2 * 2 * _LEAD < last_even[0]
            ]
            wait(len(copies) * _PAIR * _PIECE, ring.at[m % _RING])
            left -= len(copies) * _PAIR * _PIECE
        wait(left, odd_sem)

    def write_step(s, carry):
        v, r = _split(s, unit_writes)
        stream, tile = unit_of(v) * _UNIT, r * _WRITE_STEP
        copy = _window(buf, o_hbm, stream, _UNIT, tile, _WRITE_STEP)
        for t in range(0, _WRITE_STEP, _PIECE):
            copy(0, _UNIT, t, _PIECE, out_sem, 1)
        return carry

    def matmul(view, pixels):
        def at(stream, tile):
            return stream, pl.ds(tile * _ROWS, _ROWS), slice(None)

        lhs = jnp.concatenate(
            [
                jnp.concatenate([view[at(*tiles[part])] for tiles in pixels])
                for part in range(_PARTS)
            ],
            axis=1,
        )
        acc = jnp.dot(lhs, w_ref[...], preferred_element_type=jnp.float32)
        out = (acc + bias).astype(buf.dtype)
        for q, tiles in enumerate(pixels):
            for part in range(_PARTS):
                view[at(*tiles[part])] = out[
                    q * _ROWS:(q + 1) * _ROWS, part * _LANES:(part + 1) * _LANES
                ]

    def compute(v, j):
        first = [-s * _STREAM % _PARTS for s in range(_UNIT)]
        streams = pl.ds(unit_of(v) * _UNIT, _UNIT)

        @pl.when(j == jnp.where(v < groups, chunks - 1, 0))
        def _():
            matmul(buf.at[streams], [
                [divmod(s * _STREAM + first[s] - _PARTS + t, _STREAM) for t in range(_PARTS)]
                for s in range(_UNIT) if first[s]
            ])

        row = pl.multiple_of(j * (_CHUNK * _ROWS), _ROWS)
        view = buf.at[streams, pl.ds(row, (_CHUNK + rest) * _ROWS)]
        matmul(view, [
            [(s, first[s] + c + t) for t in range(_PARTS)]
            for s in range(_UNIT) for c in range(0, _CHUNK, _PARTS)
        ])

    def read_weights(turn, thread):
        rows = w_ref.shape[0] // (2 * _WEIGHT_TURNS)
        rows = pl.ds((2 * turn + thread) * rows, rows)
        copy = pltpu.make_async_copy(w_hbm.at[rows], w_ref.at[rows], out_sem)
        copy.start(priority=thread)

    for turn in range(_WEIGHT_TURNS):
        read_weights(turn, 1)
    for turn in range(_LEAD):
        if turn >= _LEAD - _WEIGHT_TURNS:
            read_weights(turn - _LEAD + _WEIGHT_TURNS, 0)
        read(2 * turn + 1)
    b_copy = pltpu.make_async_copy(b_hbm, b_ref, out_sem)
    b_copy.start()
    lax.fori_loop(0, _FIRST_READS, read_step, 0)
    pltpu.make_async_copy(w_hbm, w_ref, out_sem).wait()
    b_copy.wait()
    bias = b_ref[...].astype(jnp.float32).reshape(1, _PARTS * _LANES)

    def reads_after(done):
        return _FIRST_READS + (done * _READ_RATE >> 4)

    switch = next(i for i in range(n_matmuls) if reads_after(i) > unrolled)

    def writes_after(done):
        return _FIRST_WRITES + ((done - switch) * _WRITE_RATE >> 4)

    for done in range(switch):
        assert reads_needed(done + 1) <= min(reads_after(done + 1), unrolled)
        newest = reads_after(done + 1) + pl.cdiv(2 * _LEAD, step_copies)
        assert newest - reads_needed(done) <= _RING
    for done in range(switch, n_matmuls):
        v, tile = divmod(writes_after(done) * _WRITE_STEP - 1, _STREAM)
        assert v * chunks + min(tile // _CHUNK, chunks - 1) < done
        assert writes_after(done) <= n_writes

    def step(i, carry):
        @pl.when(i < switch)
        def _():
            hi = jnp.minimum(reads_after(i + 1), unrolled)
            lax.fori_loop(reads_after(i), hi, read_step, 0)
            pl.when(i == switch - 1)(read_last_steps)
            lax.fori_loop(reads_needed(i), reads_needed(i + 1), wait_step, 0)

        @pl.when(i == switch)
        def _():
            wait(len(on_time) * _PAIR * _PIECE, last_sem)
            lax.fori_loop(0, _FIRST_WRITES, write_step, 0)
            wait_last_steps(reads_needed(switch))

        compute(*_split(i, chunks))

        @pl.when(i >= switch)
        def _():
            hi = jnp.where(i == n_matmuls - 1, n_writes, writes_after(i + 1))
            lax.fori_loop(writes_after(i), hi, write_step, 0)

        return carry

    lax.fori_loop(0, n_matmuls, step, 0)
    pltpu.make_async_copy(buf, o_hbm, out_sem).wait()


@jax.jit
def pallas_standalone__standard_2d_1d_3d_conv__vision_kernel(
    x: jax.Array,
    w: jax.Array,
    b: jax.Array,
):
    batch, height, width, cin = x.shape
    kh, kw, _, cout = w.shape
    groups_of_8 = batch * height * width // _ROWS
    streams = groups_of_8 * _PARTS // _STREAM
    assert (kh, kw) == (1, 1) and cin == cout == _PARTS * _LANES
    assert streams * _STREAM * _ROWS * _LANES == x.size
    assert streams % (2 * _UNIT) == 0
    shape = (streams, _STREAM * _ROWS, _LANES)
    tiles = x.reshape(groups_of_8, _ROWS, _PARTS, _LANES).transpose(0, 2, 1, 3)
    hbm = pl.BlockSpec(memory_space=pltpu.HBM)
    out = pl.pallas_call(
        _conv1x1_kernel,
        in_specs=[hbm, hbm, hbm],
        out_specs=hbm,
        out_shape=jax.ShapeDtypeStruct(shape, x.dtype),
        scratch_shapes=[
            pltpu.VMEM(shape, x.dtype),
            pltpu.VMEM((cin, cout), w.dtype),
            pltpu.VMEM((cout,), b.dtype),
            pltpu.SemaphoreType.DMA((_RING,)),
            pltpu.SemaphoreType.DMA(()),
            pltpu.SemaphoreType.DMA(()),
            pltpu.SemaphoreType.DMA(()),
        ],
        compiler_params=pltpu.CompilerParams(
            vmem_limit_bytes=120 * 2**20,
            disable_bounds_checks=True,
            disable_semaphore_checks=True,
        ),
    )(tiles.reshape(shape), w.reshape(cin, cout), b)
    out = out.reshape(groups_of_8, _PARTS, _ROWS, _LANES).transpose(0, 2, 1, 3)
    return out.reshape(batch, height, width, cout)
```

```python
import jax
import jax.numpy as jnp
from jax import lax
import jax.experimental.pallas as pl
import jax.experimental.pallas.tpu as pltpu

_ROWS, _LANES = 8, 128
_PARTS = 3
_STREAM = 512
_UNIT = 6
_PIECE = 8
_CHUNK = 51

_PAIR = 2
_READ_STEP = 16
_FIRST_READS = 8
_READ_RATE = 53
_RING = 32
_LEAD = 26
_WEIGHT_TURNS = 6

_LATE = 5
_WRITE_STEP = 32
_FIRST_WRITES = 8
_WRITE_RATE = 46


def _split(i, n):
    if isinstance(i, int):
        return divmod(i, n)
    if n & (n - 1) == 0:
        return i >> (n.bit_length() - 1), i & (n - 1)
    q = lax.div(i, n)
    return q, i - q * n


def _window(src, dst, stream, streams, tile, tiles):
    row = tile * _ROWS
    if not isinstance(row, int):
        row = pl.multiple_of(row, _ROWS)
    idx = (pl.ds(stream, streams), pl.ds(row, tiles * _ROWS))
    src, dst = src.at[idx], dst.at[idx]

    def copy(stream, streams, tile, tiles, sem, thread):
        idx = (pl.ds(stream, streams), pl.ds(tile * _ROWS, tiles * _ROWS))
        pltpu.make_async_copy(src.at[idx], dst.at[idx], sem).start(priority=thread)

    return copy


def _conv1x1_kernel(
    x_hbm, w_hbm, b_hbm, o_hbm, buf, w_ref, b_ref, ring, odd_sem, last_sem, out_sem
):
    groups = buf.shape[0] // (2 * _UNIT)
    chunks, rest = divmod(_STREAM, _CHUNK)
    n_matmuls = 2 * groups * chunks
    group_reads = _STREAM // _READ_STEP
    n_reads = groups * group_reads
    unit_writes = _STREAM // _WRITE_STEP
    n_writes = 2 * groups * unit_writes

    def wait(tiles, sem):
        streams = next(
            n for n in range(1, buf.shape[0] + 1)
            if tiles % n == 0 and tiles // n <= _STREAM
        )
        size = buf.at[pl.ds(0, streams), pl.ds(0, tiles // streams * _ROWS)]
        pltpu.make_async_copy(size, size, sem).wait()

    def unit_of(v):
        return jnp.where(v < groups, 2 * v, 2 * (v - groups) + 1)

    pairs = 2 * _UNIT // _PAIR
    step_copies = pairs * _READ_STEP // _PIECE
    n_copies = n_reads * step_copies
    first_cut = n_copies + 1 - 2 * pl.cdiv(_LEAD, 3)
    unrolled = (first_cut - 2 * _LEAD) // step_copies
    last_even = range(unrolled * step_copies, n_copies, 2)
    on_time = last_even[:len(last_even) - _LATE]

    def reader(m):
        g, r = _split(m, group_reads)
        stream, tile = 2 * g * _UNIT, r * _READ_STEP
        copy = _window(x_hbm, buf, stream, 2 * _UNIT, tile, _READ_STEP)
        even_sem = ring.at[m & (_RING - 1)]

        def read(c, sem=None, quarter=None):
            piece, pair = divmod(c, pairs)
            stream, tile = pair * _PAIR, piece * _PIECE
            if sem is None:
                sem = even_sem if stream < _UNIT else odd_sem
            if quarter is None:
                copy(stream, _PAIR, tile, _PIECE, sem, c % 2)
            else:
                s, half = divmod(quarter, 2)
                copy(stream + s, 1, tile + half * _PIECE // 2, _PIECE // 2, sem, c % 2)

        return read

    def read(c, *args):
        m, c = divmod(c, step_copies)
        reader(m)(c, *args)

    def read_step(m, carry):
        readers = {}
        for c in range(step_copies):
            later, c = divmod(c + c % 2 * 2 * _LEAD, step_copies)
            if later not in readers:
                readers[later] = reader(m + later)
            readers[later](c)
        return carry

    def read_last_steps():
        odd = [(c,) for c in range(last_even[0] + 2 * _LEAD + 1, first_cut, 2)]
        odd += [(c, q) for c in range(first_cut, n_copies, 2) for q in range(4)]
        for turn, (c, *quarter) in enumerate(odd):
            if turn < len(last_even):
                even = last_even[turn]
                read(even, last_sem if even in on_time else odd_sem)
            read(c, odd_sem, *quarter)

    def reads_needed(done):
        g, j = _split(done, chunks)
        n, _ = _split(j * _CHUNK + rest + _READ_STEP - 1, _READ_STEP)
        n = n * (j > 0) if isinstance(done, int) else jnp.where(j > 0, n, 0)
        return g * group_reads + n

    def wait_step(m, carry):
        wait(_UNIT * _READ_STEP, ring.at[m & (_RING - 1)])
        return carry

    def wait_last_steps(first):
        left = buf.shape[0] * _STREAM - first * _UNIT * _READ_STEP
        left -= len(on_time) * _PAIR * _PIECE
        for m in range(first, n_reads):
            copies = [
                c for c in range(m * step_copies, (m + 1) * step_copies)
                if c % pairs * _PAIR < _UNIT and c - c % 2 * 2 * _LEAD < last_even[0]
            ]
            if copies:
                wait(len(copies) * _PAIR * _PIECE, ring.at[m % _RING])
            left -= len(copies) * _PAIR * _PIECE
        wait(left, odd_sem)

    def write_step(s, carry):
        v, r = _split(s, unit_writes)
        stream, tile = unit_of(v) * _UNIT, r * _WRITE_STEP
        copy = _window(buf, o_hbm, stream, _UNIT, tile, _WRITE_STEP)
        for t in range(0, _WRITE_STEP, _PIECE):
            copy(0, _UNIT, t, _PIECE, out_sem, 1)
        return carry

    def matmul(view, pixels):
        def at(stream, tile):
            return stream, pl.ds(tile * _ROWS, _ROWS), slice(None)

        lhs = jnp.concatenate(
            [
                jnp.concatenate([view[at(*tiles[part])] for tiles in pixels])
                for part in range(_PARTS)
            ],
            axis=1,
        )
        acc = jnp.dot(lhs, w_ref[...], preferred_element_type=jnp.float32)
        out = (acc + bias).astype(buf.dtype)
        for q, tiles in enumerate(pixels):
            for part in range(_PARTS):
                view[at(*tiles[part])] = out[
                    q * _ROWS:(q + 1) * _ROWS, part * _LANES:(part + 1) * _LANES
                ]

    def compute(v, j):
        first = [-s * _STREAM % _PARTS for s in range(_UNIT)]
        streams = pl.ds(unit_of(v) * _UNIT, _UNIT)

        @pl.when(j == jnp.where(v < groups, chunks - 1, 0))
        def _():
            matmul(buf.at[streams], [
                [divmod(s * _STREAM + first[s] - _PARTS + t, _STREAM) for t in range(_PARTS)]
                for s in range(_UNIT) if first[s]
            ])

        row = pl.multiple_of(j * (_CHUNK * _ROWS), _ROWS)
        view = buf.at[streams, pl.ds(row, (_CHUNK + rest) * _ROWS)]
        matmul(view, [
            [(s, first[s] + c + t) for t in range(_PARTS)]
            for s in range(_UNIT) for c in range(0, _CHUNK, _PARTS)
        ])

    def read_weights(turn, thread):
        rows = w_ref.shape[0] // (2 * _WEIGHT_TURNS)
        rows = pl.ds((2 * turn + thread) * rows, rows)
        copy = pltpu.make_async_copy(w_hbm.at[rows], w_ref.at[rows], out_sem)
        copy.start(priority=thread)

    for turn in range(_WEIGHT_TURNS):
        read_weights(turn, 1)
    for turn in range(_LEAD):
        if turn >= _LEAD - _WEIGHT_TURNS:
            read_weights(turn - _LEAD + _WEIGHT_TURNS, 0)
        read(2 * turn + 1)
    b_copy = pltpu.make_async_copy(b_hbm, b_ref, last_sem)
    b_copy.start()
    lax.fori_loop(0, _FIRST_READS, read_step, 0)
    pltpu.make_async_copy(w_hbm, w_ref, out_sem).wait()
    b_copy.wait()
    bias = b_ref[...].astype(jnp.float32).reshape(1, _PARTS * _LANES)

    def reads_after(done):
        return _FIRST_READS + (done * _READ_RATE >> 4)

    switch = next(i for i in range(n_matmuls) if reads_after(i) > unrolled)

    def writes_after(done):
        return _FIRST_WRITES + ((done - switch) * _WRITE_RATE >> 4)

    for done in range(switch):
        assert reads_needed(done + 1) <= min(reads_after(done + 1), unrolled)
        newest = reads_after(done + 1) + pl.cdiv(2 * _LEAD, step_copies)
        assert newest - reads_needed(done) <= _RING
    for done in range(switch, n_matmuls):
        v, tile = divmod(writes_after(done) * _WRITE_STEP - 1, _STREAM)
        assert v * chunks + min(tile // _CHUNK, chunks - 1) < done
        assert writes_after(done) <= n_writes

    def step(i, carry):
        @pl.when(i < switch)
        def _():
            hi = jnp.minimum(reads_after(i + 1), unrolled)
            lax.fori_loop(reads_after(i), hi, read_step, 0)
            pl.when(i == switch - 1)(read_last_steps)
            lax.fori_loop(reads_needed(i), reads_needed(i + 1), wait_step, 0)

        @pl.when(i == switch)
        def _():
            wait(len(on_time) * _PAIR * _PIECE, last_sem)
            lax.fori_loop(0, _FIRST_WRITES, write_step, 0)
            wait_last_steps(reads_needed(switch))

        compute(*_split(i, chunks))

        @pl.when(i >= switch)
        def _():
            hi = jnp.where(i == n_matmuls - 1, n_writes, writes_after(i + 1))
            lax.fori_loop(writes_after(i), hi, write_step, 0)

        return carry

    lax.fori_loop(0, n_matmuls, step, 0)
    pltpu.make_async_copy(buf, o_hbm, out_sem).wait()


@jax.jit
def pallas_standalone__standard_2d_1d_3d_conv__vision_kernel(
    x: jax.Array,
    w: jax.Array,
    b: jax.Array,
):
    batch, height, width, cin = x.shape
    kh, kw, _, cout = w.shape
    groups_of_8 = batch * height * width // _ROWS
    streams = groups_of_8 * _PARTS // _STREAM
    assert (kh, kw) == (1, 1) and cin == cout == _PARTS * _LANES
    assert streams * _STREAM * _ROWS * _LANES == x.size
    assert streams % (2 * _UNIT) == 0
    shape = (streams, _STREAM * _ROWS, _LANES)
    tiles = x.reshape(groups_of_8, _ROWS, _PARTS, _LANES).transpose(0, 2, 1, 3)
    hbm = pl.BlockSpec(memory_space=pltpu.HBM)
    out = pl.pallas_call(
        _conv1x1_kernel,
        in_specs=[hbm, hbm, hbm],
        out_specs=hbm,
        out_shape=jax.ShapeDtypeStruct(shape, x.dtype),
        scratch_shapes=[
            pltpu.VMEM(shape, x.dtype),
            pltpu.VMEM((cin, cout), w.dtype),
            pltpu.VMEM((cout,), b.dtype),
            pltpu.SemaphoreType.DMA((_RING,)),
            pltpu.SemaphoreType.DMA(()),
            pltpu.SemaphoreType.DMA(()),
            pltpu.SemaphoreType.DMA(()),
        ],
        compiler_params=pltpu.CompilerParams(
            vmem_limit_bytes=120 * 2**20,
            disable_bounds_checks=True,
            disable_semaphore_checks=True,
        ),
    )(tiles.reshape(shape), w.reshape(cin, cout), b)
    out = out.reshape(groups_of_8, _PARTS, _ROWS, _LANES).transpose(0, 2, 1, 3)
    return out.reshape(batch, height, width, cout)
```
